```python
import os as _os
_os.environ.setdefault("JAX_PLATFORMS", "cpu")
import jax
import jax.numpy as jnp

def _softmax(x, axis=-1):
    return jax.nn.softmax(x, axis=axis)
def _gelu(x):
    return jax.nn.gelu(x, approximate=True)
def _silu(x):
    return jax.nn.silu(x)
def _sigmoid(x):
    return jax.nn.sigmoid(x)
def _layernorm(x, axis=-1, eps=1e-5):
    m = jnp.mean(x, axis=axis, keepdims=True)
    v = jnp.var(x, axis=axis, keepdims=True)
    return (x - m) / jnp.sqrt(v + eps)
def _scatter_add(tgt, idx, src, axis=0):
    return tgt.at[idx].add(src)
def _segment_sum(src, seg, n):
    return jax.ops.segment_sum(src, seg, n)
class _Rng:
    def __init__(self, key):
        self._k = key
    def _next(self):
        self._k, sub = jax.random.split(self._k)
        return sub
    def normal(self, shape):
        return jax.random.normal(self._next(), shape, dtype=jnp.bfloat16)
    def randint(self, lo, hi, shape):
        return jax.random.randint(self._next(), shape, lo, hi, dtype=jnp.int32)
    def uniform(self, shape, lo=0.0, hi=1.0):
        return jax.random.uniform(self._next(), shape, jnp.bfloat16, lo, hi)
    def permutation(self, n):
        return jax.random.permutation(self._next(), n)


kernel_name = 'interleave_layers__gqa_block_cached__dense_activation_silu__decode'

def setup_inputs():
    _rng = _Rng(jax.random.key(int.from_bytes(__import__("os").urandom(4), "little")))
    _w = (lambda a: (lambda t: t.astype(jnp.bfloat16) if jnp.issubdtype(t.dtype, jnp.floating) else t)(jnp.asarray(a)))
    def _A_setup():
        B, Sq, D = 2, 1, 512
        Hq, Hkv, Sk, Dh = 32, 8, 8192, 128
        assert Hq % Hkv == 0, (Hq, Hkv)
        return {
            "x": _w((lambda *s: _rng.normal(s) * 0.1)(B, Sq, D)),
            "k_cache": _w((lambda *s: _rng.normal(s) * 0.8)(B, Hkv, Sk, Dh)),
            "v_cache": _w((lambda *s: _rng.normal(s) * 1.6)(B, Hkv, Sk, Dh)),
            "wq": _w((lambda *s: _rng.normal(s) * 0.8)(D, Hq * Dh) * (D ** -0.5)),
            "wo": _w((lambda *s: _rng.normal(s) * 1.6)(Hq * Dh, D) * ((Hq * Dh) ** -0.5)),
        }
    _A_in = _A_setup()

    def _B_setup():
        B, S, D, F = 2, 1, 512, 1792
        return {
            "x": _w((lambda *s: _rng.normal(s) * 0.1)(B, S, D)),
            "w1": _w((lambda *s: _rng.normal(s) * 0.4)(D, F) * (D ** -0.5)),
            "w2": _w((lambda *s: _rng.normal(s) * 0.4)(F, D) * (F ** -0.5)),
        }
    _B_in = _B_setup()

    return {
        "A_x": _A_in["x"],
        "A_k_cache": _A_in["k_cache"],
        "A_v_cache": _A_in["v_cache"],
        "A_wq": _A_in["wq"],
        "A_wo": _A_in["wo"],
        "B_x": _B_in["x"],
        "B_w1": _B_in["w1"],
        "B_w2": _B_in["w2"],
    }

def reference(A_x, A_k_cache, A_v_cache, A_wq, A_wo, B_x, B_w1, B_w2):
    def _A_ref(x, k_cache, v_cache, wq, wo):
        B, Sq, D = x.shape
        Hq, Dh = 32, 128
        Hkv = k_cache.shape[1]
        rep = Hq // Hkv
        q = (lambda x, *d: x.transpose(*d))((x @ wq).reshape(B, Sq, Hq, Dh), 0, 2, 1, 3)
        k = jnp.repeat(k_cache, rep, axis=1)
        v = jnp.repeat(v_cache, rep, axis=1)
        scores = jnp.einsum("bhqd,bhkd->bhqk", q, k) * (Dh ** -0.5)
        p = _softmax(scores, axis=-1)
        o = jnp.einsum("bhqk,bhkd->bhqd", p, v)
        return (lambda x, *d: x.transpose(*d))(o, 0, 2, 1, 3).reshape(B, Sq, Hq * Dh) @ wo

    def _B_ref(x, w1, w2):
        h = jnp.einsum("bsd,df->bsf", x, w1)
        h = _silu(h)
        out = jnp.einsum("bsf,fd->bsd", h, w2)
        return out

    x = A_x
    x = x + _A_ref(_layernorm(x, axis=-1), A_k_cache, A_v_cache, A_wq, A_wo)
    x = x + _B_ref(_layernorm(x, axis=-1), B_w1, B_w2)
    x = x + _A_ref(_layernorm(x, axis=-1), A_k_cache, A_v_cache, A_wq, A_wo)
    x = x + _B_ref(_layernorm(x, axis=-1), B_w1, B_w2)
    return x
```

```python
import jax
import jax.numpy as jnp
from jax import lax
import jax.experimental.pallas as pl
import jax.experimental.pallas.tpu as pltpu

_B, _D = 2, 512
_HQ, _HKV, _SK, _DH = 32, 8, 8192, 128
_REP = _HQ // _HKV
_GW = _REP * _DH
_F = 1792
_EPS = 1e-5
_SCALE = _DH ** -0.5

_CH = 2048
_VSPLIT = 7680
_TCH = 1024
_GATE_CHUNK = 2
_GATE_LAST = -1
_Q_GATE = 2
_NQ_MXU = 1

_KV_GROUPS = ((0, 4), (4, 2), (6, 1))
_SEM_W = 0
_SEM_G = 1
_SEM_K7, _SEM_V7A, _SEM_V7B = 4, 5, 6
_NSEM = 7
_LAST = _HKV - 1


def _kernel(x_hbm, k_hbm, v_hbm, wq_hbm, wo_hbm, w1_hbm, w2_hbm, out_ref,
            x_v, xs_scr, kst, vst, kt, vp, wq_v, wo_v, w1_v, w2_v,
            wq32, wo32, q_scr, s_scr, p_scr, y_scr, sems):
    f32, bf16, u32 = jnp.float32, jnp.bfloat16, jnp.uint32

    def group_copies(b, g):
        h0, n = _KV_GROUPS[g]
        sem = sems.at[_SEM_G + g]
        return (
            pltpu.make_async_copy(k_hbm.at[b, pl.ds(h0, n)],
                                  kst.at[pl.ds(h0, n)], sem),
            pltpu.make_async_copy(v_hbm.at[b, pl.ds(h0, n)],
                                  vst.at[pl.ds(h0, n)], sem),
        )

    def k_last_copy(b):
        return pltpu.make_async_copy(
            k_hbm.at[b, _LAST], kst.at[_LAST], sems.at[_SEM_K7])

    def v_last_copy(b, part):
        lo, n = (0, _VSPLIT) if part == 0 else (_VSPLIT, _SK - _VSPLIT)
        return pltpu.make_async_copy(
            v_hbm.at[b, _LAST, pl.ds(lo, n), :],
            vst.at[_LAST, pl.ds(lo, n), :],
            sems.at[_SEM_V7A + part])

    def start_group(b, g):
        for cp in group_copies(b, g):
            cp.start()

    def start_last(b):
        k_last_copy(b).start()
        v_last_copy(b, 0).start()
        v_last_copy(b, 1).start()

    w_copies = [
        pltpu.make_async_copy(src, dst, sems.at[_SEM_W])
        for src, dst in ((wq_hbm, wq_v), (x_hbm, x_v), (wo_hbm, wo_v),
                         (w1_hbm, w1_v), (w2_hbm, w2_v))
    ]
    for cp in w_copies:
        cp.start()
    for g in range(len(_KV_GROUPS)):
        start_group(0, g)
    start_last(0)
    for cp in w_copies:
        cp.wait()

    xf = x_v[...].astype(f32)
    for b in range(_B):
        xs_scr[b] = jnp.broadcast_to(xf[b:b + 1, :], (8, _D))

    def prep_wq(i, c):
        r0 = pl.multiple_of(i * 64, 64)
        wq32[pl.ds(r0, 64), :] = (
            wq_v[pl.ds(r0, 64), _NQ_MXU * _GW:].astype(f32))
        return c

    lax.fori_loop(0, _D // 64, prep_wq, 0)

    def prep_wo(i, c):
        r0 = pl.multiple_of(i * 256, 256)
        wo32[pl.ds(r0, 256), :] = wo_v[pl.ds(r0, 256), :].astype(f32)
        return c

    lax.fori_loop(0, _LAST * _GW // 256, prep_wo, 0)

    rowsel = lax.broadcasted_iota(jnp.int32, (8, _DH), 0)
    row128 = rowsel % _REP

    def centered(x):
        m = jnp.mean(x, axis=-1, keepdims=True)
        xc = x - m
        var = jnp.mean(xc * xc, axis=-1, keepdims=True)
        return xc, lax.rsqrt(var + _EPS)

    def rows_sum(y):
        return jnp.broadcast_to(jnp.sum(y, axis=0, keepdims=True), y.shape)

    def q_rows(qf):
        q = qf[:, 0:_DH]
        for j in range(1, _REP):
            q = jnp.where(row128 == j, qf[:, j * _DH:(j + 1) * _DH], q)
        return q.astype(bf16)

    def q_head_mxu(xcb, rstd, h):
        return q_rows(jnp.dot(xcb, wq_v[:, h * _GW:(h + 1) * _GW],
                              preferred_element_type=f32) * rstd)

    def zero_of(*vals):
        top = vals[0]
        for v in vals[1:]:
            top = jnp.maximum(top, v)
        return jnp.minimum(jnp.abs(top), 0.0)

    def gemv_vpu(xrows, w_ref, r0, c0, accs):
        xt = jnp.concatenate([xrows] * (_DH // 8), axis=0).T
        accs = list(accs)
        for g in range(_GW // 8):
            xg = xt[g * 8:(g + 1) * 8, :]
            for t in range(_REP):
                v = w_ref[r0 + g * 8:r0 + (g + 1) * 8,
                          c0 + t * _DH:c0 + (t + 1) * _DH] * xg
                accs[t] = v if accs[t] is None else accs[t] + v
        return accs

    def lane_fold(op, acc, s):
        for j in range(s.shape[1] // 128):
            t = s[:, j * 128:(j + 1) * 128]
            acc = t if acc is None else op(acc, t)
        return acc

    def qk_stream(q, h):
        mx = None
        for c in range(_SK // _TCH):
            ktc = kst[h, c * _TCH:(c + 1) * _TCH, :].T
            kt[h, :, c * _TCH:(c + 1) * _TCH] = pltpu.bitcast(ktc, u32)
            s = jnp.dot(q, ktc, preferred_element_type=f32)
            s_scr[0, :, c * _TCH:(c + 1) * _TCH] = s
            mx = lane_fold(jnp.maximum, mx, s)
        m = jnp.max(mx, axis=-1, keepdims=True)
        l = None
        for c in range(_SK // _CH):
            p = jnp.exp((s_scr[0, :, c * _CH:(c + 1) * _CH] - m) * _SCALE)
            l = lane_fold(jnp.add, l, p)
            p_scr[:, c * _CH:(c + 1) * _CH] = p.astype(bf16)
        return 1.0 / jnp.sum(l, axis=-1, keepdims=True)

    def pv_stream(h, lo, hi, o):
        c = lo
        while c < hi:
            n = min(_CH, hi - c)
            v = vst[h, c:c + n, :]
            vp[h, c // 2:(c + n) // 2, :] = pltpu.bitcast(v, u32)
            oc = jnp.dot(p_scr[:, c:c + n], v, preferred_element_type=f32)
            o = oc if o is None else o + oc
            c += n
        return o

    def qk_chunk(q, h, c, mx):
        s = jnp.dot(q, pltpu.bitcast(kt[h, :, c * _CH:(c + 1) * _CH], bf16),
                    preferred_element_type=f32)
        s_scr[h, :, c * _CH:(c + 1) * _CH] = s
        return lane_fold(jnp.maximum, mx, s)

    def pv_chunk(m, h, c, o, l, zero=None):
        s = s_scr[h, :, c * _CH:(c + 1) * _CH]
        if zero is not None:
            s = jnp.concatenate([s[:, :128] + zero, s[:, 128:]], axis=1)
        p = jnp.exp((s - m) * _SCALE)
        l = lane_fold(jnp.add, l, p)
        v = pltpu.bitcast(vp[h, c * _CH // 2:(c + 1) * _CH // 2, :], bf16)
        oc = jnp.dot(p.astype(bf16), v, preferred_element_type=f32)
        return (oc if o is None else o + oc), l

    def flat_rows(o):
        return jnp.concatenate(
            [jnp.broadcast_to(o[j:j + 1, :], (8, _DH)) for j in range(_REP)],
            axis=1)

    def out_proj_mxu(o, wo_rows):
        return jnp.dot(flat_rows(o).astype(bf16), wo_rows,
                       preferred_element_type=f32)

    def ffn(x):
        xc, rstd = centered(x)
        hid = jnp.dot(xc.astype(bf16), w1_v[...],
                      preferred_element_type=f32) * rstd
        hid = hid * jax.nn.sigmoid(hid)
        return x + jnp.dot(hid.astype(bf16), w2_v[...],
                           preferred_element_type=f32)

    def batch_body(b, carry):
        x0 = xs_scr[b]

        xc, rstd = centered(x0)
        xcb = xc.astype(bf16)
        for h in range(_HKV):
            q_scr[h] = q_head_mxu(xcb, rstd, h)
        y_scr[...] = x0

        def head_body(h, c2):
            for g, (h0, n) in enumerate(_KV_GROUPS):
                @pl.when(h == h0)
                def _():
                    for cp in group_copies(b, g):
                        cp.wait()

            rl = qk_stream(q_scr[h], h)
            o = pv_stream(h, 0, _SK, None)
            r0 = pl.multiple_of(h * _GW, _GW)
            y_scr[...] += out_proj_mxu(o * rl, wo_v[pl.ds(r0, _GW), :])

            for g, (h0, n) in enumerate(_KV_GROUPS):
                @pl.when(jnp.logical_and(h == h0 + n - 1, b == 0))
                def _():
                    start_group(1, g)
            return c2

        lax.fori_loop(0, _LAST, head_body, 0)

        k_last_copy(b).wait()
        rl = qk_stream(q_scr[_LAST], _LAST)
        v_last_copy(b, 0).wait()
        o = pv_stream(_LAST, 0, _VSPLIT, None)
        v_last_copy(b, 1).wait()
        o = pv_stream(_LAST, _VSPLIT, _SK, o)

        @pl.when(b == 0)
        def _():
            start_last(1)

        x1 = y_scr[...] + out_proj_mxu(o * rl, wo_v[_LAST * _GW:, :])
        x2 = ffn(x1)

        xc, rstd = centered(x2)
        xcb = xc.astype(bf16)
        qs = [None] * _HKV
        for h in range(_NQ_MXU):
            qs[h] = q_head_mxu(xcb, rstd, h)
        xn = xc * rstd

        nch = _SK // _CH

        def qk(h):
            mx = None
            firsts = []
            for c in range(nch):
                mx = qk_chunk(qs[h], h, c, mx)
                firsts.append(mx)
            return jnp.max(mx, axis=-1, keepdims=True), firsts

        def q_head_vpu(h, gate):
            xg = xn
            if gate is not None:
                xg = xn + jnp.concatenate([zero_of(gate)] * _REP, axis=1)
            accs = gemv_vpu(xg, wq32, 0, (h - _NQ_MXU) * _GW, [None] * _REP)
            return q_rows(rows_sum(jnp.concatenate(accs, axis=1)))

        ms = [None] * _HKV
        os_ = [None] * _HKV
        yaccs = [None] * _REP
        for h in range(_NQ_MXU, 2):
            qs[h] = q_head_vpu(h, None)
        ms[0], _ = qk(0)
        for h in range(_HKV):
            if h + 1 < _HKV:
                ms[h + 1], gates = qk(h + 1)
            zero = None
            if h >= 1:
                yaccs = gemv_vpu(flat_rows(os_[h - 1]), wo32, (h - 1) * _GW,
                                 0, yaccs)
                zero = zero_of(*yaccs)
            if h + 2 < _HKV and h + 2 >= _NQ_MXU:
                qs[h + 2] = q_head_vpu(h + 2, gates[_Q_GATE])
            o = l = None
            for c in range(nch):
                gc = _GATE_CHUNK if h < _LAST else _GATE_LAST
                o, l = pv_chunk(ms[h], h, c, o, l, zero if c == gc else None)
            os_[h] = o / jnp.sum(l, axis=-1, keepdims=True)
        x3 = x2 + rows_sum(jnp.concatenate(yaccs, axis=1))
        x3 = x3 + out_proj_mxu(os_[_LAST], wo_v[_LAST * _GW:, :])
        xs_scr[b] = ffn(x3)
        return carry

    lax.fori_loop(0, _B, batch_body, 0)
    row2 = lax.broadcasted_iota(jnp.int32, (_B, _D), 0)
    out_ref[...] = jnp.where(row2 == 0, xs_scr[0, 0:_B, :],
                             xs_scr[1, 0:_B, :]).astype(out_ref.dtype)


@jax.jit
def pallas_interleave_layers__gqa_block_cached__dense_activation_silu__decode_kernel(
    A_x: jax.Array,
    A_k_cache: jax.Array,
    A_v_cache: jax.Array,
    A_wq: jax.Array,
    A_wo: jax.Array,
    B_x: jax.Array,
    B_w1: jax.Array,
    B_w2: jax.Array,
):
    del B_x
    bf16, f32, u32 = jnp.bfloat16, jnp.float32, jnp.uint32
    any_spec = pl.BlockSpec(memory_space=pl.ANY)
    out = pl.pallas_call(
        _kernel,
        out_shape=jax.ShapeDtypeStruct((_B, _D), A_x.dtype),
        in_specs=[any_spec] * 7,
        out_specs=pl.BlockSpec(memory_space=pltpu.VMEM),
        scratch_shapes=[
            pltpu.VMEM((_B, _D), bf16),
            pltpu.VMEM((_B, 8, _D), f32),
            pltpu.VMEM((_HKV, _SK, _DH), bf16),
            pltpu.VMEM((_HKV, _SK, _DH), bf16),
            pltpu.VMEM((_HKV, _DH // 2, _SK), u32),
            pltpu.VMEM((_HKV, _SK // 2, _DH), u32),
            pltpu.VMEM((_D, _HQ * _DH), bf16),
            pltpu.VMEM((_HQ * _DH, _D), bf16),
            pltpu.VMEM((_D, _F), bf16),
            pltpu.VMEM((_F, _D), bf16),
            pltpu.VMEM((_D, (_HKV - _NQ_MXU) * _GW), f32),
            pltpu.VMEM((_LAST * _GW, _D), f32),
            pltpu.VMEM((_HKV, 8, _DH), bf16),
            pltpu.VMEM((_HKV, 8, _SK), f32),
            pltpu.VMEM((8, _SK), bf16),
            pltpu.VMEM((8, _D), f32),
            pltpu.SemaphoreType.DMA((_NSEM,)),
        ],
        compiler_params=pltpu.CompilerParams(
            vmem_limit_bytes=110 * 1024 * 1024),
    )(A_x.reshape(_B, _D), A_k_cache, A_v_cache, A_wq, A_wo, B_w1, B_w2)
    return out.reshape(A_x.shape)
```

```python
import jax
import jax.numpy as jnp
from jax import lax
import jax.experimental.pallas as pl
import jax.experimental.pallas.tpu as pltpu

_B, _D = 2, 512
_HQ, _HKV, _SK, _DH = 32, 8, 8192, 128
_REP = _HQ // _HKV
_GW = _REP * _DH
_F = 1792
_EPS = 1e-5
_SCALE = _DH ** -0.5
_LAST = _HKV - 1

_CH = 2048
_TCH = 512
_SCH = 1024
_VCH = 1024
_C1 = 512
_R2 = 768
_GATE_CHUNK = 2
_Q_GATE = 2
_NQ_MXU = 1

_NQR = 4
_QR = _SK // _NQR
_LOR = 512
_VS1 = 1536
_VS2 = 1920
_VCUTS = (0, _VS1, _VS2, _QR)
_TK = 128
_NTK = _SK // _TK
_PACE = 64
_KT0 = 3
_VHI = 32
_EK = _SK // _TCH
_ES = _SK // _SCH
_EV = _SK // _VCH
_T1A = 0
_T1 = 22
_T2 = 10
_PREP_PACE = 20
_NOCHK = False

_SEM_W = 0
_SEM_K = 1
_SEM_V = _SEM_K + _HKV
_NSEM = _SEM_V + _LAST + len(_VCUTS) - 1


def _check_tick_plan():
    n = _EK + _ES
    for h in range(_LAST):
        n += 0 if h < 2 else (_T1A if h == 2 else _T1)
        assert n >= (h + 2 - _KT0) * _NTK, (h, n)
        n += _EK + _ES + (0 if h < 2 else _T2) + _EV
    assert (_VHI // _NQR) * _TK % _LOR == 0 and _VS1 % _LOR == 0
    assert (_NTK, _HKV, _NQR) == (64, 8, 4)


_check_tick_plan()


def _kernel(x_hbm, k_hbm, v_hbm, wq_hbm, wo_hbm, w1_hbm, w2_hbm, out_ref,
            x_v, xs_scr, stg, kt, vp, wq_v, wo_v, w1_v, w2_v,
            wq32, wo32, w1_32, w2_32, w1p, w2p, wqp, wop, cs_q, cs_1,
            q_scr, st_scr, s_scr, p_scr, l_scr, y_scr, sems):
    f32, bf16, u32 = jnp.float32, jnp.bfloat16, jnp.uint32
    kst = stg.at[pl.ds(0, _HKV)]
    vst = stg.at[pl.ds(_HKV, _HKV)]

    def k_copy(b, h, lo=0, hi=_QR):
        return pltpu.make_async_copy(
            k_hbm.at[b, h, :, pl.ds(lo, hi - lo), :],
            kst.at[h, :, pl.ds(lo, hi - lo), :], sems.at[_SEM_K + h])

    def v_copy(b, h, lo=0, hi=_QR, part=0):
        return pltpu.make_async_copy(
            v_hbm.at[b, h, :, pl.ds(lo, hi - lo), :],
            vst.at[h, :, pl.ds(lo, hi - lo), :], sems.at[_SEM_V + h + part])

    def bulk_k(b, h):
        for r in range(0, _QR, _LOR):
            k_copy(b, h, r, r + _LOR).start(priority=1)

    def bulk_v(b, h, lo=0, hi=_QR):
        for r in range(lo, hi, _LOR):
            v_copy(b, h, r, r + _LOR).start(priority=1)

    def tick(src, dst, sem0, item):
        h = (item >> 6) & (_HKV - 1)
        qr = item & (_NQR - 1)
        r0 = pl.multiple_of((item & (_NTK - _NQR)) * (_TK // _NQR), _TK)
        pltpu.make_async_copy(src.at[item >> 9, h, qr, pl.ds(r0, _TK), :],
                              dst.at[h, qr, pl.ds(r0, _TK), :],
                              sems.at[sem0 + h]).start(priority=0)

    def k_tick(item):
        tick(k_hbm, kst, _SEM_K, item)

    def paced(lo, hi, fn):
        def body(i, c):
            fn(i)
            pl.delay(_PACE)
            return c
        lax.fori_loop(lo, hi, body, 0)

    w_copies = [
        pltpu.make_async_copy(src, dst, sems.at[_SEM_W])
        for src, dst in ((wq_hbm, wq_v), (x_hbm, x_v), (w1_hbm, w1_v),
                         (wo_hbm, wo_v), (w2_hbm, w2_v))
    ]
    for cp in w_copies[:3]:
        cp.start(priority=1)
    bulk_v(0, 0)
    bulk_k(0, 2)
    bulk_v(0, 1)

    def w_tick(src, dst, i, rows):
        r0 = pl.multiple_of(i * rows, rows)
        pltpu.make_async_copy(src.at[pl.ds(r0, rows), :],
                              dst.at[pl.ds(r0, rows), :],
                              sems.at[_SEM_W]).start(priority=0)

    def w_ticks(i):
        w_tick(wo_hbm, wo_v, i, 32)
        pl.delay(_PACE)
        w_tick(wo_hbm, wo_v, i + 64, 32)

        @pl.when(i < _F // 32)
        def _():
            pl.delay(_PACE)
            w_tick(w2_hbm, w2_v, i, 32)

    paced(0, 64, w_ticks)
    paced(0, _NTK, k_tick)
    for cp in w_copies:
        cp.wait()

    def prep_a(i, c):
        k_tick(_NTK + i)
        r0 = pl.multiple_of(i * 16, 16)
        p0 = pl.multiple_of(i * 8, 8)
        wq32[pl.ds(r0, 16), :] = (
            wq_v[pl.ds(r0, 16), _NQ_MXU * _GW:].astype(f32))
        wqp[pl.ds(p0, 8), :] = pltpu.bitcast(
            wq_v[pl.ds(r0, 16), :_NQ_MXU * _GW], u32)
        w1_32[pl.ds(r0, 16), :] = w1_v[pl.ds(r0, 16), :_C1].astype(f32)
        w1p[pl.ds(p0, 8), :] = pltpu.bitcast(w1_v[pl.ds(r0, 16), _C1:], u32)
        pl.delay(_PREP_PACE)
        return c

    lax.fori_loop(0, _D // 16, prep_a, 0)

    def prep_b(i, c):
        k_tick(_NTK + _D // 16 + i)
        r0 = pl.multiple_of(i * 128, 128)
        n_wo = _LAST * _GW // 128

        @pl.when(i < n_wo)
        def _():
            wo32[pl.ds(r0, 128), :] = wo_v[pl.ds(r0, 128), :].astype(f32)

        @pl.when(i >= n_wo)
        def _():
            p0 = pl.multiple_of((i - n_wo) * 64, 64)
            wop[pl.ds(p0, 64), :] = pltpu.bitcast(wo_v[pl.ds(r0, 128), :], u32)

        r2 = pl.multiple_of(i * 64, 64)
        na, nb, nc = _C1 // 64, (_C1 + _R2) // 64, _F // 64

        @pl.when(i < na)
        def _():
            p0 = pl.multiple_of((nc - nb + i) * 32, 32)
            w2p[pl.ds(p0, 32), :] = pltpu.bitcast(w2_v[pl.ds(r2, 64), :], u32)

        @pl.when(jnp.logical_and(i >= na, i < nb))
        def _():
            d0 = pl.multiple_of((i - na) * 64, 64)
            w2_32[pl.ds(d0, 64), :] = w2_v[pl.ds(r2, 64), :].astype(f32)

        @pl.when(jnp.logical_and(i >= nb, i < nc))
        def _():
            p0 = pl.multiple_of((i - nb) * 32, 32)
            w2p[pl.ds(p0, 32), :] = pltpu.bitcast(w2_v[pl.ds(r2, 64), :], u32)
        return c

    lax.fori_loop(0, _HQ * _DH // 128, prep_b, 0)

    ones = jnp.ones((8, _D), bf16)
    cs_q[...] = jnp.dot(ones, wq_v[:, :_NQ_MXU * _GW],
                        preferred_element_type=f32)
    cs_1[...] = jnp.dot(ones, w1_v[...], preferred_element_type=f32)

    rowsel = lax.broadcasted_iota(jnp.int32, (8, _DH), 0)
    row128 = rowsel % _REP

    def lane_fold(op, acc, s):
        for j in range(s.shape[1] // 128):
            t = s[:, j * 128:(j + 1) * 128]
            acc = t if acc is None else op(acc, t)
        return acc

    def ln_stats(x, shift=None):
        xb = x.astype(bf16)
        xr = xb.astype(f32)
        if shift is None:
            m = jnp.mean(xr, axis=-1, keepdims=True)
            xc = xr - m
            var = jnp.mean(xc * xc, axis=-1, keepdims=True)
        else:
            d = xr - shift
            both = jnp.where(rowsel < 4, lane_fold(jnp.add, None, d),
                             lane_fold(jnp.add, None, d * d))
            r = jnp.sum(both, axis=-1, keepdims=True) * (1.0 / _D)
            s1 = jnp.broadcast_to(r[0:1, :], (8, 1))
            s2 = jnp.broadcast_to(r[4:5, :], (8, 1))
            m = shift + s1
            xc = None
            var = jnp.maximum(s2 - s1 * s1, 0.0)
        return xb, xc, m, lax.rsqrt(var + _EPS)

    def rows_sum(y):
        return jnp.broadcast_to(jnp.sum(y, axis=0, keepdims=True), y.shape)

    def q_rows(qf):
        q = qf[:, 0:_DH]
        for j in range(1, _REP):
            q = jnp.where(row128 == j, qf[:, j * _DH:(j + 1) * _DH], q)
        return q.astype(bf16)

    def zero_of(*vals):
        top = vals[0]
        for v in vals[1:]:
            top = jnp.maximum(top, v)
        return jnp.minimum(jnp.abs(top), 0.0)

    def gemv_vpu(xrows, w_ref, r0, c0, accs):
        xt = jnp.concatenate([xrows] * (_DH // 8), axis=0).T
        xt = xt.astype(f32)
        accs = list(accs)
        for g in range(xrows.shape[1] // 8):
            xg = xt[g * 8:(g + 1) * 8, :]
            for t in range(len(accs)):
                v = w_ref[r0 + g * 8:r0 + (g + 1) * 8,
                          c0 + t * _DH:c0 + (t + 1) * _DH] * xg
                accs[t] = v if accs[t] is None else accs[t] + v
        return accs

    def pv_stream(h, slot, lo, hi, o, emit=None):
        e = 0
        for qr in range(_NQR):
            for r in range(lo, hi, _VCH):
                r1 = min(r + _VCH, hi)
                if emit is not None:
                    emit(e)
                    e += 1
                c0, c1 = qr * _QR + r, qr * _QR + r1
                v = vst[h, qr, r:r1, :]
                vp[h, c0 // 2:c1 // 2, :] = pltpu.bitcast(v, u32)
                p = jnp.concatenate(
                    [p_scr[slot, c // _SCH, :, c % _SCH:c % _SCH + 128]
                     for c in range(c0, c1, 128)], axis=1)
                oc = jnp.dot(p, v, preferred_element_type=f32)
                o = oc if o is None else o + oc
        return o

    def qk_chunk(q, h, c, mx):
        s = jnp.dot(q, pltpu.bitcast(kt[h, :, c * _CH:(c + 1) * _CH], bf16),
                    preferred_element_type=f32)
        s_scr[h, :, c * _CH:(c + 1) * _CH] = s
        return lane_fold(jnp.maximum, mx, s)

    def pv_chunk(m, sc, h, c, o, l, zero=None):
        s = s_scr[h, :, c * _CH:(c + 1) * _CH]
        if zero is not None:
            s = jnp.concatenate([s[:, :128] + zero, s[:, 128:]], axis=1)
        p = jnp.exp((s - m) * sc)
        l = lane_fold(jnp.add, l, p)
        v = pltpu.bitcast(vp[h, c * _CH // 2:(c + 1) * _CH // 2, :], bf16)
        oc = jnp.dot(p.astype(bf16), v, preferred_element_type=f32)
        return (oc if o is None else o + oc), l

    def flat_rows(o):
        return jnp.concatenate(
            [jnp.broadcast_to(o[j:j + 1, :], (8, _DH)) for j in range(_REP)],
            axis=1)

    def out_proj_mxu(o, wo_rows):
        return jnp.dot(flat_rows(o).astype(bf16), wo_rows,
                       preferred_element_type=f32)

    def ffn(x, shift):
        xb, _, m, rstd = ln_stats(x, shift)

        def act(pre, lo, hi):
            half = (pre - m * cs_1[:, lo:hi]) * (0.5 * rstd)
            return half * jnp.tanh(half) + half

        h_m = act(jnp.dot(xb, pltpu.bitcast(w1p[...], bf16),
                          preferred_element_type=f32), _C1, _F).astype(bf16)
        h_v = act(rows_sum(jnp.concatenate(
            gemv_vpu(xb, w1_32, 0, 0, [None] * (_C1 // _DH)), axis=1)),
            0, _C1).astype(bf16)
        y_v = rows_sum(jnp.concatenate(
            gemv_vpu(h_m[:, :_R2], w2_32, 0, 0, [None] * (_D // _DH)), axis=1))
        y_m = jnp.dot(jnp.concatenate([h_m[:, _R2:], h_v], axis=1),
                      pltpu.bitcast(w2p[...], bf16),
                      preferred_element_type=f32)
        return (x + y_v) + y_m

    xf = x_v[...].astype(f32)
    x_rows = [jnp.broadcast_to(xf[b:b + 1, :], (8, _D)) for b in range(_B)]
    row512 = lax.broadcasted_iota(jnp.int32, (8, _D), 0)
    _, xc, mu, rstd = ln_stats(jnp.where(row512 < 4, x_rows[0], x_rows[1]))
    xcb = xc.astype(bf16)
    stats = jnp.where(lax.broadcasted_iota(jnp.int32, (8, _DH), 1) == 0,
                      mu, rstd * _SCALE)
    for b in range(_B):
        xs_scr[b] = x_rows[b]
        st_scr[b] = jnp.broadcast_to(stats[4 * b:4 * b + 1, :], (8, _DH))
    for h in range(_HKV):
        qf = jnp.dot(xcb, wq_v[:, h * _GW:(h + 1) * _GW],
                     preferred_element_type=f32)
        for b in range(_B):
            q_scr[b, h] = q_rows(
                jnp.broadcast_to(qf[4 * b:4 * b + 1, :], (8, _GW)))

    def batch_body(b, carry):
        y_scr[...] = xs_scr[b]
        mu = st_scr[b, :, 0:1]
        sc = st_scr[b, :, 1:2]

        item0 = (b * _HKV + _KT0) * _NTK
        n_k = jnp.where(b == 0, (_HKV + 1) * _NTK, _B * _HKV * _NTK)
        n_all = jnp.where(b == 0, n_k, n_k + _VHI)

        def any_tick(n):
            @pl.when(n < n_k)
            def _():
                k_tick(n)

            @pl.when(jnp.logical_and(n >= n_k, n < n_all))
            def _():
                tick(v_hbm, vst, _SEM_V, n - _NTK)

        def idle(n, count):
            paced(n, jnp.minimum(n + count, n_all), any_tick)
            return n + count

        def k_phase(h, n):
            slot = h & 1
            k_copy(b, h).wait()
            q = q_scr[b, h]
            mx = None
            for c in range(_SK // _TCH):
                any_tick(n + c)
                r0 = (c * _TCH) % _QR
                ktc = kst[h, c * _TCH // _QR, r0:r0 + _TCH, :].T
                kt[h, :, c * _TCH:(c + 1) * _TCH] = pltpu.bitcast(ktc, u32)
                s = jnp.dot(q, ktc, preferred_element_type=f32)
                c0 = (c * _TCH) % _SCH
                s_scr[c * _TCH // _SCH, :, c0:c0 + _TCH] = s
                mx = lane_fold(jnp.maximum, mx, s)
            n = n + _EK

            def soft(c, l):
                any_tick(n + c)
                m = jnp.max(mx, axis=-1, keepdims=True)
                p = jnp.exp((s_scr[c, :, 0:_SCH] - m) * sc)
                p_scr[slot, c] = p.astype(bf16)
                return lane_fold(jnp.add, l, p)

            l_scr[slot] = lax.fori_loop(0, _ES, soft,
                                        jnp.zeros((8, _DH), f32))
            return n + _ES

        def recip_l(slot):
            return 1.0 / jnp.sum(l_scr[slot], axis=-1, keepdims=True)

        def step(h, n):
            n = idle(n, jnp.where(h < 2, 0, jnp.where(h == 2, _T1A, _T1)))
            n = k_phase(h + 1, n)
            n = idle(n, jnp.where(h < 2, 0, _T2))
            v_copy(b, h).wait()
            o = pv_stream(h, h & 1, 0, _QR, None, lambda e: any_tick(n + e))
            r0 = pl.multiple_of(h * _GW, _GW)
            y_scr[...] += out_proj_mxu(o * recip_l(h & 1),
                                       wo_v[pl.ds(r0, _GW), :])

            @pl.when(h < _LAST - 3)
            def _():
                bulk_v(b, jnp.minimum(h + 3, _LAST - 1))

            @pl.when(h == _LAST - 3)
            def _():
                front = (_VHI // _NQR) * _TK

                @pl.when(b == 0)
                def _():
                    bulk_v(b, _LAST, 0, front)

                bulk_v(b, _LAST, front, _VS1)
                for part in range(1, len(_VCUTS) - 1):
                    v_copy(b, _LAST, _VCUTS[part], _VCUTS[part + 1],
                           part).start(priority=1)

            @pl.when(jnp.logical_and(h == _LAST - 2, b == 0))
            def _():
                bulk_k(1, 1)

            @pl.when(jnp.logical_and(h == _LAST - 1, b == 0))
            def _():
                bulk_v(1, 0)
            return n + _EV

        bulk_v(b, 2)
        n = k_phase(b * 0, item0)
        n = lax.fori_loop(0, _LAST, step, n)
        paced(n, n_all, any_tick)

        rl = recip_l(_LAST % 2)
        o = None
        for part in range(len(_VCUTS) - 1):
            v_copy(b, _LAST, _VCUTS[part], _VCUTS[part + 1], part).wait()
            o = pv_stream(_LAST, _LAST % 2, _VCUTS[part], _VCUTS[part + 1], o)

        @pl.when(b == 0)
        def _():
            bulk_k(1, 2)
            bulk_v(1, 1)

        x1 = y_scr[...] + out_proj_mxu(o * rl, pltpu.bitcast(wop[...], bf16))
        x2 = ffn(x1, mu)

        xb, xn, mu, rstd = ln_stats(x2)
        sc = rstd * _SCALE
        qs = [None] * _HKV
        for h in range(_NQ_MXU):
            qf = jnp.dot(xb, pltpu.bitcast(wqp[:, h * _GW:(h + 1) * _GW], bf16),
                         preferred_element_type=f32)
            qs[h] = q_rows(qf - mu * cs_q[:, h * _GW:(h + 1) * _GW])

        nch = _SK // _CH

        def qk(h):
            mx = None
            firsts = []
            for c in range(nch):
                mx = qk_chunk(qs[h], h, c, mx)
                firsts.append(mx)
            return jnp.max(mx, axis=-1, keepdims=True), firsts

        def q_head_vpu(h, gate):
            xg = xn
            if gate is not None:
                xg = xn + jnp.concatenate([zero_of(gate)] * _REP, axis=1)
            accs = gemv_vpu(xg, wq32, 0, (h - _NQ_MXU) * _GW, [None] * _REP)
            return q_rows(rows_sum(jnp.concatenate(accs, axis=1)))

        ms = [None] * _HKV
        os_ = [None] * _HKV
        yaccs = [None] * _REP
        for h in range(_NQ_MXU, 2):
            qs[h] = q_head_vpu(h, None)
        ms[0], _ = qk(0)
        for h in range(_HKV):
            if h + 1 < _HKV:
                ms[h + 1], gates = qk(h + 1)
            zero = None
            if h >= 1:
                yaccs = gemv_vpu(flat_rows(os_[h - 1]), wo32, (h - 1) * _GW,
                                 0, yaccs)
                zero = zero_of(*yaccs)
            if h + 2 < _HKV and h + 2 >= _NQ_MXU:
                qs[h + 2] = q_head_vpu(h + 2, gates[_Q_GATE])
            o = l = None
            for c in range(nch):
                gated = h < _LAST and c == _GATE_CHUNK
                o, l = pv_chunk(ms[h], sc, h, c, o, l, zero if gated else None)
            os_[h] = o / jnp.sum(l, axis=-1, keepdims=True)
        x3 = x2 + rows_sum(jnp.concatenate(yaccs, axis=1))
        x3 = x3 + out_proj_mxu(os_[_LAST], pltpu.bitcast(wop[...], bf16))
        xs_scr[b] = ffn(x3, mu)
        return carry

    lax.fori_loop(0, _B, batch_body, 0)
    row2 = lax.broadcasted_iota(jnp.int32, (_B, _D), 0)
    out_ref[...] = jnp.where(row2 == 0, xs_scr[0, 0:_B, :],
                             xs_scr[1, 0:_B, :]).astype(out_ref.dtype)


@jax.jit
def pallas_interleave_layers__gqa_block_cached__dense_activation_silu__decode_kernel(
    A_x: jax.Array,
    A_k_cache: jax.Array,
    A_v_cache: jax.Array,
    A_wq: jax.Array,
    A_wo: jax.Array,
    B_x: jax.Array,
    B_w1: jax.Array,
    B_w2: jax.Array,
):
    del B_x
    bf16, f32, u32 = jnp.bfloat16, jnp.float32, jnp.uint32
    any_spec = pl.BlockSpec(memory_space=pl.ANY)
    kv_shape = (_B, _HKV, _NQR, _QR, _DH)
    out = pl.pallas_call(
        _kernel,
        out_shape=jax.ShapeDtypeStruct((_B, _D), A_x.dtype),
        in_specs=[any_spec] * 7,
        out_specs=pl.BlockSpec(memory_space=pltpu.VMEM),
        scratch_shapes=[
            pltpu.VMEM((_B, _D), bf16),
            pltpu.VMEM((_B, 8, _D), f32),
            pltpu.VMEM((2 * _HKV, _NQR, _QR, _DH), bf16),
            pltpu.VMEM((_HKV, _DH // 2, _SK), u32),
            pltpu.VMEM((_HKV, _SK // 2, _DH), u32),
            pltpu.VMEM((_D, _HQ * _DH), bf16),
            pltpu.VMEM((_HQ * _DH, _D), bf16),
            pltpu.VMEM((_D, _F), bf16),
            pltpu.VMEM((_F, _D), bf16),
            pltpu.VMEM((_D, (_HKV - _NQ_MXU) * _GW), f32),
            pltpu.VMEM((_LAST * _GW, _D), f32),
            pltpu.VMEM((_D, _C1), f32),
            pltpu.VMEM((_R2, _D), f32),
            pltpu.VMEM((_D // 2, _F - _C1), u32),
            pltpu.VMEM(((_F - _R2) // 2, _D), u32),
            pltpu.VMEM((_D // 2, _NQ_MXU * _GW), u32),
            pltpu.VMEM((_GW // 2, _D), u32),
            pltpu.VMEM((8, _NQ_MXU * _GW), f32),
            pltpu.VMEM((8, _F), f32),
            pltpu.VMEM((_B, _HKV, 8, _DH), bf16),
            pltpu.VMEM((_B, 8, _DH), f32),
            pltpu.VMEM((_HKV, 8, _SK), f32),
            pltpu.VMEM((2, _ES, 8, _SCH), bf16),
            pltpu.VMEM((2, 8, _DH), f32),
            pltpu.VMEM((8, _D), f32),
            pltpu.SemaphoreType.DMA((_NSEM,)),
        ],
        compiler_params=pltpu.CompilerParams(
            vmem_limit_bytes=110 * 1024 * 1024,
            disable_bounds_checks=_NOCHK),
    )(A_x.reshape(_B, _D), A_k_cache.reshape(kv_shape),
      A_v_cache.reshape(kv_shape), A_wq, A_wo, B_w1, B_w2)
    return out.reshape(A_x.shape)
```

```python
import jax
import jax.numpy as jnp
from jax import lax
import jax.experimental.pallas as pl
import jax.experimental.pallas.tpu as pltpu

_B, _D = 2, 512
_HQ, _HKV, _SK, _DH = 32, 8, 8192, 128
_REP = _HQ // _HKV
_GW = _REP * _DH
_F = 1792
_EPS = 1e-5
_SCALE = _DH ** -0.5
_LAST = _HKV - 1

_CH = 2048
_TCH = 512
_SCH = 1024
_VCH = 1024
_C1 = 384
_W2V = tuple(_C1 // 128 + t for t in (0, 1, 4, 5, 6, 7))
_W2M = tuple(t for t in (*range(_C1 // 128, _F // 128), *range(_C1 // 128))
             if t not in _W2V)
_R2 = 128 * len(_W2V)
_NVS = (4, 4, 4, 4, 4, 4, 4, 0)
_NV = max(_NVS)
_GATE_CHUNK = 2
_Q_GATE = 2
_NQ_MXU = 1

_NQR = 4
_QR = _SK // _NQR
_LOR = 256
_LOSH = 112
_VS1 = 1536
_VS2 = 1920
_VCUTS = (0, _VS1, _VS2, _QR)
_TK = 128
_NTK = _SK // _TK
_TSH = _LOSH % _TK
_PACE = 63
_KT0 = 3
_VHI = 8
_EK = _SK // _TCH
_ES = _SK // _SCH
_EV = _SK // _VCH
_T1A = 0
_T1 = 22
_T2 = 10
_PREP_PACE = 20
_WOR = _HQ * _DH // 4
_WOSH = 32
_WO_AHEAD = 12
_WQC = 1792
_PIN_LAG = 2

_SEM_W = 0
_SEM_K = 1
_SEM_V = _SEM_K + _HKV
_NSEM = _SEM_V + _LAST + len(_VCUTS) - 1


def _check_tick_plan():
    n = _EK + _ES
    for h in range(_LAST):
        n += 0 if h < 2 else (_T1A if h == 2 else _T1)
        assert n >= (h + 2 - _KT0) * _NTK, (h, n)
        n += _EK + _ES + (0 if h < 2 else _T2) + _EV
    assert _VHI % (2 * _NQR) == 0 and _TSH + (_VHI // _NQR) * _TK <= _VS1
    assert 0 < _TSH < _TK and _TSH % 16 == 0
    assert (_NTK, _HKV, _NQR) == (64, 8, 4)


_check_tick_plan()


def _kernel(x_hbm, k_hbm, v_hbm, wq_hbm, wo_hbm, w1_hbm, w2_hbm, out_ref,
            x_v, xs_scr, stg, kt, kt32, vp, wq_v, wo_v, w1_v, w2_v,
            wq32, wo32, w1_32, w2_32, w1p, w2p, wqp, wop, cs_q, cs_1,
            q_scr, st_scr, s_scr, p_scr, l_scr, y_scr, sems):
    f32, bf16, u32 = jnp.float32, jnp.bfloat16, jnp.uint32
    kst = stg.at[pl.ds(0, _HKV)]
    vst = stg.at[pl.ds(_HKV, _HKV)]
    spare = stg.at[2 * _HKV, 0]

    def k_copy(b, h, lo=0, hi=_QR):
        return pltpu.make_async_copy(
            k_hbm.at[b, h, :, pl.ds(lo, hi - lo), :],
            kst.at[h, :, pl.ds(lo, hi - lo), :], sems.at[_SEM_K + h])

    def v_copy(b, h, lo=0, hi=_QR, part=0):
        return pltpu.make_async_copy(
            v_hbm.at[b, h, :, pl.ds(lo, hi - lo), :],
            vst.at[h, :, pl.ds(lo, hi - lo), :], sems.at[_SEM_V + h + part])

    def pieces(lo, hi):
        cuts = [lo] + [r for r in range(_LOSH, _QR, _LOR) if lo < r < hi] + [hi]
        return zip(cuts[:-1], cuts[1:])

    def bulk_k(b, h):
        for r0, r1 in pieces(0, _QR):
            k_copy(b, h, r0, r1).start(priority=1)

    def bulk_v(b, h, lo=0, hi=_QR):
        for r0, r1 in pieces(lo, hi):
            v_copy(b, h, r0, r1).start(priority=1)

    def tick(src, dst, sem0, item):
        h = (item >> 6) & (_HKV - 1)
        qr = (item >> 1) & 3
        idx = ((item >> 2) & 14) | (item & 1)
        r0 = pl.multiple_of(idx * _TK + _TSH, 16)
        pltpu.make_async_copy(src.at[item >> 9, h, qr, pl.ds(r0, _TK), :],
                              dst.at[h, qr, pl.ds(r0, _TK), :],
                              sems.at[sem0 + h]).start(priority=0)

    def k_tick(item, ok=None):
        real = (item & 57) != 57
        if ok is not None:
            real = jnp.logical_and(real, ok)

        @pl.when(real)
        def _():
            tick(k_hbm, kst, _SEM_K, item)

    def k_edges(b, h):
        k_copy(b, h, 0, _TSH).start(priority=0)
        k_copy(b, h, _QR - _TK + _TSH, _QR).start(priority=0)

    def paced(lo, hi, fn):
        def body(i, c):
            fn(i)
            pl.delay(_PACE)
            return c
        lax.fori_loop(lo, hi, body, 0)

    w_copies = [
        pltpu.make_async_copy(src, dst, sems.at[_SEM_W])
        for src, dst in ((x_hbm, x_v), (w1_hbm, w1_v), (wq_hbm, wq_v),
                         (wo_hbm, wo_v), (w2_hbm, w2_v))
    ]

    def wo_bulk(r0, n):
        pltpu.make_async_copy(wo_hbm.at[:, pl.ds(r0, n), :],
                              wo_v.at[:, pl.ds(r0, n), :],
                              sems.at[_SEM_W]).start(priority=1)

    wo_cuts = [0, *range(_WOSH, _WOR, 64), _WOR]
    wo_pieces = list(zip(wo_cuts[:-1], wo_cuts[1:]))
    for r0, r1 in wo_pieces[:_WO_AHEAD]:
        wo_bulk(r0, r1 - r0)
    w_copies[0].start(priority=1)

    def wq_ticks(i):
        g = (i & 3) * 16 + (i >> 2)
        r0 = pl.multiple_of(g * 8, 8)
        r1 = pl.multiple_of(((g + 1) & 63) * 8, 8)
        n_hi = _HQ * _DH - _WQC
        pltpu.make_async_copy(wq_hbm.at[pl.ds(r0, 8), pl.ds(_WQC, n_hi)],
                              wq_v.at[pl.ds(r0, 8), pl.ds(_WQC, n_hi)],
                              sems.at[_SEM_W]).start(priority=0)
        pl.delay(_PACE)
        pltpu.make_async_copy(wq_hbm.at[pl.ds(r1, 8), pl.ds(0, _WQC)],
                              wq_v.at[pl.ds(r1, 8), pl.ds(0, _WQC)],
                              sems.at[_SEM_W]).start(priority=0)

    def w_tick(src, dst, i, rows):
        r0 = pl.multiple_of(i * rows, rows)
        pltpu.make_async_copy(src.at[pl.ds(r0, rows), :],
                              dst.at[pl.ds(r0, rows), :],
                              sems.at[_SEM_W]).start(priority=0)

    def w2_ticks(i):
        p = (i & 1) * 14 + (i >> 1)
        w_tick(w2_hbm, w2_v, 2 * p + 1, 32)
        pl.delay(_PACE)
        w_tick(w2_hbm, w2_v, jnp.where(2 * p + 2 == _F // 32, 0, 2 * p + 2), 32)

    paced(0, 24, wq_ticks)
    for r0, r1 in wo_pieces[_WO_AHEAD:]:
        wo_bulk(r0, r1 - r0)
    w_copies[1].start(priority=1)
    paced(24, 64, wq_ticks)
    bulk_v(0, 0)
    paced(0, _F // 64, w2_ticks)
    bulk_k(0, 2)
    k_edges(0, 0)
    paced(0, _NTK, k_tick)
    k_edges(0, 1)
    for cp in w_copies:
        cp.wait()

    def prep_a(i, c):
        k_tick(_NTK + i)
        r0 = pl.multiple_of(i * 16, 16)
        p0 = pl.multiple_of(i * 8, 8)
        wq32[pl.ds(r0, 16), :] = (
            wq_v[pl.ds(r0, 16), _NQ_MXU * _GW:].astype(f32))
        wqp[pl.ds(p0, 8), :] = pltpu.bitcast(
            wq_v[pl.ds(r0, 16), :_NQ_MXU * _GW], u32)
        w1_32[pl.ds(r0, 16), :] = w1_v[pl.ds(r0, 16), :_C1].astype(f32)
        w1p[pl.ds(p0, 8), :] = pltpu.bitcast(w1_v[pl.ds(r0, 16), _C1:], u32)
        pl.delay(_PREP_PACE)
        return c

    lax.fori_loop(0, _D // 16, prep_a, 0)
    bulk_v(0, 1)

    def prep_b(i, c):
        k_tick(_NTK + _D // 16 + i)
        r0 = pl.multiple_of(i * 128, 128)
        n_wo = _LAST * _GW // 128

        def wo_blk():
            return wo_v[i >> 3, pl.ds(pl.multiple_of((i & 7) * 128, 128), 128), :]

        @pl.when(i < n_wo)
        def _():
            wo32[pl.ds(r0, 128), :] = wo_blk().astype(f32)

        @pl.when(i >= n_wo)
        def _():
            p0 = pl.multiple_of((i - n_wo) * 64, 64)
            wop[pl.ds(p0, 64), :] = pltpu.bitcast(wo_blk(), u32)

        return c - 1

    zero_s = lax.fori_loop(0, _HQ * _DH // 128, prep_b, 32)

    for i, t in enumerate(_W2V):
        w2_32[i * 128:(i + 1) * 128, :] = (
            w2_v[t * 128:(t + 1) * 128, :].astype(f32))
    for i, t in enumerate(_W2M):
        w2p[i * 64:(i + 1) * 64, :] = pltpu.bitcast(
            w2_v[t * 128:(t + 1) * 128, :], u32)

    ones = jnp.ones((8, _D), bf16)
    cs_q[...] = jnp.dot(ones, wq_v[:, :_NQ_MXU * _GW],
                        preferred_element_type=f32)
    cs_1[...] = jnp.dot(ones, w1_v[...], preferred_element_type=f32)

    rowsel = lax.broadcasted_iota(jnp.int32, (8, _DH), 0)
    row128 = rowsel % _REP

    def lane_fold(op, acc, s):
        for j in range(s.shape[1] // 128):
            t = s[:, j * 128:(j + 1) * 128]
            acc = t if acc is None else op(acc, t)
        return acc

    def ln_stats(x, shift):
        xb = (x - shift).astype(bf16)
        xr = xb.astype(f32)
        both = jnp.where(rowsel < 4, lane_fold(jnp.add, None, xr),
                         lane_fold(jnp.add, None, xr * xr))
        r = jnp.sum(both, axis=-1, keepdims=True) * (1.0 / _D)
        m = jnp.broadcast_to(r[0:1, :], (8, 1))
        s2 = jnp.broadcast_to(r[4:5, :], (8, 1))
        var = jnp.maximum(s2 - m * m, 0.0)
        return xb, xr, m, lax.rsqrt(var + _EPS)

    def rows_sum(y):
        return jnp.broadcast_to(jnp.sum(y, axis=0, keepdims=True), y.shape)

    def q_rows(qf):
        q = qf[:, 0:_DH]
        for j in range(1, _REP):
            q = jnp.where(row128 == j, qf[:, j * _DH:(j + 1) * _DH], q)
        return q.astype(bf16)

    def zero_of(*vals):
        top = vals[0]
        for v in vals[1:]:
            top = jnp.maximum(top, v)
        return jnp.minimum(jnp.abs(top), 0.0)

    def gemv_vpu(xrows, w_ref, r0, c0, accs):
        xt = jnp.concatenate([xrows] * (_DH // 8), axis=0).T
        xt = xt.astype(f32)
        accs = list(accs)
        for g in range(xrows.shape[1] // 8):
            xg = xt[g * 8:(g + 1) * 8, :]
            for t in range(len(accs)):
                v = w_ref[r0 + g * 8:r0 + (g + 1) * 8,
                          c0 + t * _DH:c0 + (t + 1) * _DH] * xg
                accs[t] = v if accs[t] is None else accs[t] + v
        return accs

    def pv_stream(h, slot, lo, hi, o, emit=None):
        e = 0
        for qr in range(_NQR):
            for r in range(lo, hi, _VCH):
                r1 = min(r + _VCH, hi)
                if emit is not None:
                    emit(e)
                    e += 1
                c0, c1 = qr * _QR + r, qr * _QR + r1
                v = vst[h, qr, r:r1, :]
                vp[h, c0 // 2:c1 // 2, :] = pltpu.bitcast(v, u32)
                p = jnp.concatenate(
                    [p_scr[slot, c // _SCH, :, c % _SCH:c % _SCH + 128]
                     for c in range(c0, c1, 128)], axis=1)
                oc = jnp.dot(p, v, preferred_element_type=f32)
                o = oc if o is None else o + oc
        return o

    def qk_chunk(q, h, c, mx, hook, skm):
        lo, hi = c * _CH, min((c + 1) * _CH, skm)
        s = jnp.dot(hook(q), pltpu.bitcast(kt[h, :, lo:hi], bf16),
                    preferred_element_type=f32)
        s_scr[h, :, lo:hi] = s
        return lane_fold(jnp.maximum, mx, s)

    def qk_vpu(q, h, mx):
        qf = q.astype(f32)
        nvh = _NVS[h]
        rowv = lax.broadcasted_iota(jnp.int32, (8, nvh * 128), 0) % _REP
        s = None
        for j in range(_REP):
            qj = jnp.broadcast_to(qf[j:j + 1, :], (8, _DH))
            sj = rows_sum(jnp.concatenate(
                gemv_vpu(qj, kt32.at[h + zero_s * (j + 1)], 0,
                         (_NV - nvh) * 128, [None] * nvh), axis=1))
            s = sj if s is None else jnp.where(rowv == j, sj, s)
        s_scr[h, :, _SK - nvh * 128:] = s
        return lane_fold(jnp.maximum, mx, s)

    def pv_chunk(m, sc, h, c, o, l, zero, hook):
        s = s_scr[h, :, c * _CH:(c + 1) * _CH]
        if zero is not None:
            s = jnp.concatenate([s[:, :128] + zero, s[:, 128:]], axis=1)
        p = jnp.exp((s - m) * sc)
        l = lane_fold(jnp.add, l, p)
        v = pltpu.bitcast(vp[h, c * _CH // 2:(c + 1) * _CH // 2, :], bf16)
        oc = jnp.dot(hook(p.astype(bf16)), v, preferred_element_type=f32)
        return (oc if o is None else o + oc), l

    def flat_rows(o):
        return jnp.concatenate(
            [jnp.broadcast_to(o[j:j + 1, :], (8, _DH)) for j in range(_REP)],
            axis=1)

    def out_proj_mxu(o, wo_rows):
        return jnp.dot(flat_rows(o).astype(bf16), wo_rows,
                       preferred_element_type=f32)

    def ffn(x, shift):
        xb, _, m, rstd = ln_stats(x, shift)

        def act(pre, lo, hi):
            half = (pre - m * cs_1[:, lo:hi]) * (0.5 * rstd)
            return half * jnp.tanh(half) + half

        h_m = act(jnp.dot(xb, pltpu.bitcast(w1p[...], bf16),
                          preferred_element_type=f32), _C1, _F).astype(bf16)
        h_v = act(rows_sum(jnp.concatenate(
            gemv_vpu(xb, w1_32, 0, 0, [None] * (_C1 // _DH)), axis=1)),
            0, _C1).astype(bf16)
        hid = jnp.concatenate([h_v, h_m], axis=1)

        def tiles(ts):
            return jnp.concatenate(
                [hid[:, t * 128:(t + 1) * 128] for t in ts], axis=1)

        y_v = rows_sum(jnp.concatenate(
            gemv_vpu(tiles(_W2V), w2_32, 0, 0, [None] * (_D // _DH)), axis=1))
        y_m = jnp.dot(tiles(_W2M), pltpu.bitcast(w2p[...], bf16),
                      preferred_element_type=f32)
        return (x + y_v) + y_m, shift + m

    xf = x_v[...].astype(f32)
    x_rows = [jnp.broadcast_to(xf[b:b + 1, :], (8, _D)) for b in range(_B)]
    row512 = lax.broadcasted_iota(jnp.int32, (8, _D), 0)
    xin = jnp.where(row512 < 4, x_rows[0], x_rows[1])
    mu = jnp.mean(xin, axis=-1, keepdims=True)
    xc = xin - mu
    rstd = lax.rsqrt(jnp.mean(xc * xc, axis=-1, keepdims=True) + _EPS)
    xcb = xc.astype(bf16)
    stats = jnp.where(lax.broadcasted_iota(jnp.int32, (8, _DH), 1) == 0,
                      mu, rstd * _SCALE)
    for b in range(_B):
        xs_scr[b] = x_rows[b]
        st_scr[b] = jnp.broadcast_to(stats[4 * b:4 * b + 1, :], (8, _DH))
    for h in range(_HKV):
        qf = jnp.dot(xcb, wq_v[:, h * _GW:(h + 1) * _GW],
                     preferred_element_type=f32)
        for b in range(_B):
            q_scr[b, h] = q_rows(
                jnp.broadcast_to(qf[4 * b:4 * b + 1, :], (8, _GW)))

    def batch_body(b):
        nv = _NV if b == _B - 1 else 0
        skm = _SK - nv * 128
        y_scr[...] = xs_scr[b]
        mu = st_scr[b, :, 0:1]
        sc = st_scr[b, :, 1:2]

        item0 = (b * _HKV + _KT0) * _NTK
        n_k = (_HKV + 1) * _NTK if b == 0 else _B * _HKV * _NTK

        def any_tick(n):
            k_tick(n, n < n_k)

        def idle(n, count):
            paced(n, jnp.minimum(n + count, n_k), k_tick)
            return n + count

        def k_phase(h, n):
            slot = h & 1
            k_copy(b, h).wait()
            q = q_scr[b, h]
            mx = None
            for c in range(_SK // _TCH):
                any_tick(n + c)
                r0 = (c * _TCH) % _QR
                ktc = kst[h, c * _TCH // _QR, r0:r0 + _TCH, :].T
                kt[h, :, c * _TCH:(c + 1) * _TCH] = pltpu.bitcast(ktc, u32)
                lo = max(c * _TCH, skm)
                if lo < (c + 1) * _TCH:
                    kt32[h, :, lo - skm:(c + 1) * _TCH - skm] = (
                        ktc[:, lo - c * _TCH:].astype(f32))
                s = jnp.dot(q, ktc, preferred_element_type=f32)
                c0 = (c * _TCH) % _SCH
                s_scr[c * _TCH // _SCH, :, c0:c0 + _TCH] = s
                mx = lane_fold(jnp.maximum, mx, s)
            n = n + _EK

            def soft(c, l):
                any_tick(n + c)
                m = jnp.max(mx, axis=-1, keepdims=True)
                p = jnp.exp((s_scr[c, :, 0:_SCH] - m) * sc)
                p_scr[slot, c] = p.astype(bf16)
                return lane_fold(jnp.add, l, p)

            l_scr[slot] = lax.fori_loop(0, _ES, soft,
                                        jnp.zeros((8, _DH), f32))
            return n + _ES

        def recip_l(slot):
            return 1.0 / jnp.sum(l_scr[slot], axis=-1, keepdims=True)

        def step(h, n):
            n = idle(n, jnp.where(h < 2, 0, jnp.where(h == 2, _T1A, _T1)))
            if b > 0:
                v0 = n_k - _NTK
                paced(v0, jnp.where(h == _LAST - 1, v0 + _VHI, v0),
                      lambda i: tick(v_hbm, vst, _SEM_V, i))
            n = k_phase(h + 1, n)
            n = idle(n, jnp.where(h < 2, 0, _T2))
            v_copy(b, h).wait()
            o = pv_stream(h, h & 1, 0, _QR, None, lambda e: any_tick(n + e))
            r0 = pl.multiple_of((h & 1) * _GW, _GW)
            y_scr[...] += out_proj_mxu(o * recip_l(h & 1),
                                       wo_v[h >> 1, pl.ds(r0, _GW), :])

            @pl.when(jnp.logical_and(h != 1, h < _LAST - 2))
            def _():
                bulk_v(b, jnp.where(h == 0, 3, jnp.minimum(h + 2, _LAST - 1)))

            @pl.when(h == _LAST - 2)
            def _():
                front = 0
                if b > 0:
                    front = _TSH + (_VHI // _NQR) * _TK
                    bulk_v(b, _LAST, 0, _TSH)
                bulk_v(b, _LAST, front, _VS1)
                for part in range(1, len(_VCUTS) - 1):
                    v_copy(b, _LAST, _VCUTS[part], _VCUTS[part + 1],
                           part).start(priority=1)

            @pl.when(h + _KT0 + 1 <= _LAST)
            def _():
                k_edges(b, jnp.minimum(h + _KT0 + 1, _LAST))

            if b == 0:
                @pl.when(h == _LAST - 1)
                def _():
                    bulk_v(1, 0)
                    k_edges(1, 0)
            return n + _EV

        if b > 0:
            bulk_v(b, 1)
        n = k_phase(zero_s, item0 + zero_s)
        bulk_v(b, 2)
        k_edges(b, _KT0)
        n = lax.fori_loop(0, _LAST, step, n)
        paced(n, n_k, k_tick)

        rl = recip_l(_LAST % 2)
        o = None
        for part in range(len(_VCUTS) - 1):
            v_copy(b, _LAST, _VCUTS[part], _VCUTS[part + 1], part).wait()
            o = pv_stream(_LAST, _LAST % 2, _VCUTS[part], _VCUTS[part + 1], o)

        if b == 0:
            bulk_k(1, 2)
            k_edges(1, 1)

        x1 = y_scr[...] + out_proj_mxu(o * rl, pltpu.bitcast(wop[...], bf16))
        x2, mu = ffn(x1, mu)

        xb, xr, m2, rstd = ln_stats(x2, mu)
        xn = xr - m2
        mu = mu + m2
        sc = rstd * _SCALE
        qs = [None] * _HKV
        for h in range(_NQ_MXU):
            qf = jnp.dot(xb, pltpu.bitcast(wqp[:, h * _GW:(h + 1) * _GW], bf16),
                         preferred_element_type=f32)
            qs[h] = q_rows(qf - m2 * cs_q[:, h * _GW:(h + 1) * _GW])

        nch = _SK // _CH

        results = []

        def hook(lhs):
            i = len(results)
            if b != 0:
                return lhs
            t = lhs[:, :128]
            if i >= _PIN_LAG:
                t = (t.astype(f32) + zero_of(results[i - _PIN_LAG])).astype(bf16)
            spare[i * 16:i * 16 + 8, :] = t
            k_tick(n_k + zero_s + i)
            t = spare[i * 16:i * 16 + 8, :]
            if lhs.shape[1] == 128:
                return t
            return jnp.concatenate([t, lhs[:, 128:]], axis=1)

        def qk(h):
            mx = None
            firsts = []
            for c in range(nch):
                mx = qk_chunk(qs[h], h, c, mx, hook,
                              _SK - (_NVS[h] * 128 if nv else 0))
                results.append(mx)
                firsts.append(mx)
            if nv and _NVS[h]:
                mx = qk_vpu(qs[h], h, mx)
            return jnp.max(mx, axis=-1, keepdims=True), firsts

        def q_head_vpu(h, gate):
            xg = xn
            if gate is not None:
                xg = xn + jnp.concatenate([zero_of(gate)] * _REP, axis=1)
            accs = gemv_vpu(xg, wq32, 0, (h - _NQ_MXU) * _GW, [None] * _REP)
            return q_rows(rows_sum(jnp.concatenate(accs, axis=1)))

        ms = [None] * _HKV
        os_ = [None] * _HKV
        yaccs = [None] * _REP
        for h in range(_NQ_MXU, 2):
            qs[h] = q_head_vpu(h, None)
        ms[0], _ = qk(0)
        for h in range(_HKV):
            if h + 1 < _HKV:
                ms[h + 1], gates = qk(h + 1)
            zero = None
            if h >= 1:
                yaccs = gemv_vpu(flat_rows(os_[h - 1]), wo32, (h - 1) * _GW,
                                 0, yaccs)
                zero = zero_of(*yaccs)
            if h + 2 < _HKV and h + 2 >= _NQ_MXU:
                qs[h + 2] = q_head_vpu(h + 2, gates[_Q_GATE])
            o = l = None
            for c in range(nch):
                gated = h < _LAST and c == _GATE_CHUNK
                o, l = pv_chunk(ms[h], sc, h, c, o, l,
                                zero if gated else None, hook)
                results.append(o)
            os_[h] = o / jnp.sum(l, axis=-1, keepdims=True)
        x3 = x2 + rows_sum(jnp.concatenate(yaccs, axis=1))
        x3 = x3 + out_proj_mxu(os_[_LAST], pltpu.bitcast(wop[...], bf16))
        assert len(results) == _NTK
        xs_scr[b] = ffn(x3, mu)[0]

    for b in range(_B):
        batch_body(b)
    row2 = lax.broadcasted_iota(jnp.int32, (_B, _D), 0)
    out_ref[...] = jnp.where(row2 == 0, xs_scr[0, 0:_B, :],
                             xs_scr[1, 0:_B, :]).astype(out_ref.dtype)


@jax.jit
def pallas_interleave_layers__gqa_block_cached__dense_activation_silu__decode_kernel(
    A_x: jax.Array,
    A_k_cache: jax.Array,
    A_v_cache: jax.Array,
    A_wq: jax.Array,
    A_wo: jax.Array,
    B_x: jax.Array,
    B_w1: jax.Array,
    B_w2: jax.Array,
):
    del B_x
    bf16, f32, u32 = jnp.bfloat16, jnp.float32, jnp.uint32
    any_spec = pl.BlockSpec(memory_space=pl.ANY)
    kv_shape = (_B, _HKV, _NQR, _QR, _DH)
    extra = {}
    if hasattr(pltpu.CompilerParams, "disable_semaphore_checks"):
        extra["disable_semaphore_checks"] = True
    out = pl.pallas_call(
        _kernel,
        out_shape=jax.ShapeDtypeStruct((_B, _D), A_x.dtype),
        in_specs=[any_spec] * 7,
        out_specs=pl.BlockSpec(memory_space=pltpu.VMEM),
        scratch_shapes=[
            pltpu.VMEM((_B, _D), bf16),
            pltpu.VMEM((_B, 8, _D), f32),
            pltpu.VMEM((2 * _HKV + 1, _NQR, _QR, _DH), bf16),
            pltpu.VMEM((_HKV, _DH // 2, _SK), u32),
            pltpu.VMEM((_HKV, _DH, _NV * 128), f32),
            pltpu.VMEM((_HKV, _SK // 2, _DH), u32),
            pltpu.VMEM((_D, _HQ * _DH), bf16),
            pltpu.VMEM((4, _WOR, _D), bf16),
            pltpu.VMEM((_D, _F), bf16),
            pltpu.VMEM((_F, _D), bf16),
            pltpu.VMEM((_D, (_HKV - _NQ_MXU) * _GW), f32),
            pltpu.VMEM((_LAST * _GW, _D), f32),
            pltpu.VMEM((_D, _C1), f32),
            pltpu.VMEM((_R2, _D), f32),
            pltpu.VMEM((_D // 2, _F - _C1), u32),
            pltpu.VMEM(((_F - _R2) // 2, _D), u32),
            pltpu.VMEM((_D // 2, _NQ_MXU * _GW), u32),
            pltpu.VMEM((_GW // 2, _D), u32),
            pltpu.VMEM((8, _NQ_MXU * _GW), f32),
            pltpu.VMEM((8, _F), f32),
            pltpu.VMEM((_B, _HKV, 8, _DH), bf16),
            pltpu.VMEM((_B, 8, _DH), f32),
            pltpu.VMEM((_HKV, 8, _SK), f32),
            pltpu.VMEM((2, _ES, 8, _SCH), bf16),
            pltpu.VMEM((2, 8, _DH), f32),
            pltpu.VMEM((8, _D), f32),
            pltpu.SemaphoreType.DMA((_NSEM,)),
        ],
        compiler_params=pltpu.CompilerParams(
            vmem_limit_bytes=110 * 1024 * 1024, **extra),
    )(A_x.reshape(_B, _D), A_k_cache.reshape(kv_shape),
      A_v_cache.reshape(kv_shape), A_wq, A_wo.reshape(4, _WOR, _D), B_w1, B_w2)
    return out.reshape(A_x.shape)
```
